```python
import os as _os
_os.environ.setdefault("JAX_PLATFORMS", "cpu")
import jax
import jax.numpy as jnp

def _softmax(x, axis=-1):
    return jax.nn.softmax(x, axis=axis)
def _gelu(x):
    return jax.nn.gelu(x, approximate=True)
def _silu(x):
    return jax.nn.silu(x)
def _sigmoid(x):
    return jax.nn.sigmoid(x)
def _layernorm(x, axis=-1, eps=1e-5):
    m = jnp.mean(x, axis=axis, keepdims=True)
    v = jnp.var(x, axis=axis, keepdims=True)
    return (x - m) / jnp.sqrt(v + eps)
def _scatter_add(tgt, idx, src, axis=0):
    return tgt.at[idx].add(src)
def _segment_sum(src, seg, n):
    return jax.ops.segment_sum(src, seg, n)
class _Rng:
    def __init__(self, key):
        self._k = key
    def _next(self):
        self._k, sub = jax.random.split(self._k)
        return sub
    def normal(self, shape):
        return jax.random.normal(self._next(), shape, dtype=jnp.bfloat16)
    def randint(self, lo, hi, shape):
        return jax.random.randint(self._next(), shape, lo, hi, dtype=jnp.int32)
    def uniform(self, shape, lo=0.0, hi=1.0):
        return jax.random.uniform(self._next(), shape, jnp.bfloat16, lo, hi)
    def permutation(self, n):
        return jax.random.permutation(self._next(), n)


kernel_name = 'interleave_layers__grouped_kv_mqa__sliding_block__prompt'

def setup_inputs():
    _rng = _Rng(jax.random.key(int.from_bytes(__import__("os").urandom(4), "little")))
    _w = (lambda a: (lambda t: t.astype(jnp.bfloat16) if jnp.issubdtype(t.dtype, jnp.floating) else t)(jnp.asarray(a)))
    def _A_setup():
        B, S, D, H = 1, 2048, 448, 16
        Dh = D // H
        return {
            "x": _w((lambda *s: _rng.normal(s) * 0.05)(B, S, D)),
            "wq": _w((lambda *s: _rng.normal(s) * 0.05)(D, H * Dh)),
            "wk": _w((lambda *s: _rng.normal(s) * 0.05)(D, Dh)),
            "wv": _w((lambda *s: _rng.normal(s) * 0.05)(D, Dh)),
            "wo": _w((lambda *s: _rng.normal(s) * 0.05)(H * Dh, D)),
        }
    _A_in = _A_setup()

    def _B_setup():
        B, S, D = 1, 2048, 448
        return {
            "x": _w((lambda *s: _rng.normal(s) * 0.05)(B, S, D)),
            "wqkv": _w((lambda *s: _rng.normal(s) * 0.05)(D, 3 * D)),
            "wo": _w((lambda *s: _rng.normal(s) * 0.05)(D, D)),
        }
    _B_in = _B_setup()

    return {
        "A_x": _A_in["x"],
        "A_wq": _A_in["wq"],
        "A_wk": _A_in["wk"],
        "A_wv": _A_in["wv"],
        "A_wo": _A_in["wo"],
        "B_x": _B_in["x"],
        "B_wqkv": _B_in["wqkv"],
        "B_wo": _B_in["wo"],
    }

def reference(A_x, A_wq, A_wk, A_wv, A_wo, B_x, B_wqkv, B_wo):
    def _A_ref(x, wq, wk, wv, wo):
        B, S, D = x.shape
        H = 16
        Dh = D // H
        q = (lambda x, *d: x.transpose(*d))((x @ wq).reshape(B, S, H, Dh), 0, 2, 1, 3)
        k = x @ wk
        v = x @ wv
        scores = jnp.einsum("bhqd,bkd->bhqk", q, k) * (Dh ** -0.5)
        p = _softmax(scores, axis=-1)
        o = jnp.einsum("bhqk,bkd->bhqd", p, v)
        return (lambda x, *d: x.transpose(*d))(o, 0, 2, 1, 3).reshape(B, S, H * Dh) @ wo

    def _B_ref(x, wqkv, wo):
        B, S, D = x.shape
        H = 16; Dh = D // H; W = 256
        qkv = (lambda x, *d: x.transpose(*d))((x @ wqkv).reshape(B, S, 3, H, Dh), 2, 0, 3, 1, 4)
        q, k, v = qkv[0], qkv[1], qkv[2]
        scores = jnp.einsum("bhqd,bhkd->bhqk", q, k) * (Dh ** -0.5)
        idx = jnp.arange(S)
        mask = (idx[:, None] - idx[None, :] >= 0) & (idx[:, None] - idx[None, :] < W)
        scores = jnp.where(mask[None, None], scores, -1e9)
        p = _softmax(scores, axis=-1)
        o = jnp.einsum("bhqk,bhkd->bhqd", p, v)
        return (lambda x, *d: x.transpose(*d))(o, 0, 2, 1, 3).reshape(B, S, D) @ wo

    x = A_x
    x = x + _A_ref(_layernorm(x, axis=-1), A_wq, A_wk, A_wv, A_wo)
    x = x + _B_ref(_layernorm(x, axis=-1), B_wqkv, B_wo)
    x = x + _A_ref(_layernorm(x, axis=-1), A_wq, A_wk, A_wv, A_wo)
    x = x + _B_ref(_layernorm(x, axis=-1), B_wqkv, B_wo)
    return x
```

```python
import jax
import jax.numpy as jnp
import numpy as np
from jax import lax
import jax.experimental.pallas as pl
import jax.experimental.pallas.tpu as pltpu

S, D, H, DH, WIN = 2048, 448, 16, 28, 256
HP = 32
TB = 512
NB = S // TB
CK = 128
NC = S // CK
U = 4
UB = 2
QSCALE = float(DH ** -0.5 * np.log2(np.e))
F32, BF16 = jnp.float32, jnp.bfloat16


def _mm(a, b):
    return jnp.dot(a, b, preferred_element_type=F32)


def _layernorm_t(x):
    mean = jnp.sum(x, axis=0, keepdims=True) * (1.0 / D)
    xc = x - mean
    var = jnp.sum(xc * xc, axis=0, keepdims=True) * (1.0 / D)
    return (xc * lax.rsqrt(var + 1e-5)).astype(BF16)


def _pad_heads_t(w):
    w = w.astype(F32)
    z = jnp.zeros((HP - DH, D), F32)
    parts = []
    for h in range(H):
        parts += [w[h * DH:(h + 1) * DH], z]
    return jnp.concatenate(parts, axis=0).T.astype(BF16)


def _kernel(xt_ref, wq_ref, wkt_ref, wvt_ref, wo_ref, wqkv_ref, bwo_ref, out_ref,
            x_s, wa_s, woa_s, wb_s, wob_s, q_s, ka_s, va_s, o_s, m_s, s_s, kb_s, vb_s, mb_s):
    wa_s[0:D, :] = wq_ref[...].astype(F32).T.astype(BF16)
    z = jnp.zeros((HP - DH, D), F32)
    wa_s[D:D + 2 * HP, :] = jnp.concatenate(
        [wkt_ref[...].astype(F32), z, wvt_ref[...].astype(F32), z], axis=0).astype(BF16)
    woa_s[...] = _pad_heads_t(wo_ref[...])
    wb_s[...] = wqkv_ref[...].astype(F32).T.astype(BF16)
    wob_s[...] = _pad_heads_t(bwo_ref[...])
    for b in range(NB):
        x_s[b] = xt_ref[:, b * TB:(b + 1) * TB].astype(F32)

    row = lax.broadcasted_iota(jnp.int32, (HP, TB), 0)
    ones_row = jnp.where(row == DH, 1.0, 0.0).astype(F32)

    def a_proj(b, _):
        y = _mm(wa_s[...], _layernorm_t(x_s[b]))
        for h in range(H):
            q_s[b * H + h] = (y[h * DH:h * DH + HP] * QSCALE).astype(BF16)
        t0 = pl.multiple_of(b * TB, TB)
        ka_s[pl.ds(t0, TB), :] = y[D:D + HP].T.astype(BF16)
        va_s[b] = (y[D + HP:D + 2 * HP] + ones_row).astype(BF16)
        return _

    def scores(c, q, u, m8):
        s = _mm(ka_s[c * CK:(c + 1) * CK, :], q)
        s_s[u, c * CK:(c + 1) * CK, :] = s
        cm = jnp.max(s.reshape(CK // 8, 8, TB), axis=0)
        return cm if m8 is None else jnp.maximum(m8, cm)

    def values(c, m, u, acc):
        p = jnp.exp2(s_s[u, c * CK:(c + 1) * CK, :] - m).astype(BF16)
        per = TB // CK
        d = _mm(va_s[c // per, :, (c % per) * CK:(c % per + 1) * CK], p)
        return d if acc is None else acc + d

    def a_step(t, u, do_values, do_scores):
        acc = m8 = None
        if do_values:
            m = m_s[u, 0:1, :]
        if do_scores:
            q = q_s[t + U if do_values else t]
        for c in range(NC):
            if do_values:
                acc = values(c, m, u, acc)
            if do_scores:
                m8 = scores(c, q, u, m8)
        if do_values:
            o = acc * (1.0 / acc[DH:DH + 1, :])
            o_s[t // H, pl.ds(pl.multiple_of((t % H) * HP, HP), HP), :] = o.astype(BF16)
        if do_scores:
            m_s[u, 0:1, :] = jnp.max(m8, axis=0, keepdims=True)

    def a_attn():
        for u in range(U):
            a_step(u, u, False, True)

        def body(i, _):
            for u in range(U):
                a_step(i * U + u, u, True, True)
            return _
        lax.fori_loop(0, NB * H // U - 1, body, None)
        for u in range(U):
            a_step(NB * H - U + u, u, True, False)

    def a_out_b_proj(b, _):
        x = x_s[b] + _mm(woa_s[...], o_s[b])
        x_s[b] = x
        y = _mm(wb_s[...], _layernorm_t(x))
        t0 = pl.multiple_of(b * TB, TB)
        for h in range(H):
            q_s[b * H + h] = (y[h * DH:h * DH + HP] * QSCALE).astype(BF16)
            k = jnp.where(row < DH, y[D + h * DH:D + h * DH + HP], 0.0)
            kb_s[h, pl.ds(t0, TB), :] = k.T.astype(BF16)
            lo = min(2 * D + h * DH, 3 * D - HP)
            v = y[lo:lo + HP]
            if lo != 2 * D + h * DH:
                v = pltpu.roll(v, HP - (2 * D + h * DH - lo), axis=0)
            vb_s[b * H + h] = jnp.where(row < DH, v, ones_row).astype(BF16)
        return _

    kk = lax.broadcasted_iota(jnp.int32, (CK, CK), 0)
    qq = lax.broadcasted_iota(jnp.int32, (CK, CK), 1)
    causal = kk <= qq

    PER = TB // CK

    def b_scores(h, i, u):
        b, c = i // PER, i % PER
        q = q_s[b * H + h, :, c * CK:(c + 1) * CK]
        j0 = max(i - 2, 0)
        s = _mm(kb_s[h, j0 * CK:(i + 1) * CK, :], q)
        edge = jnp.where(causal, s[(i - j0) * CK:], s[0:CK] if i >= 2 else -jnp.inf)
        r0 = 2 * CK * b
        s_s[u, r0:r0 + CK, c * CK:(c + 1) * CK] = edge
        m = jnp.max(edge.reshape(CK // 8, 8, CK), axis=0)
        if i >= 1:
            mid = s[(i - 1 - j0) * CK:(i - j0) * CK]
            s_s[u, r0 + CK:r0 + 2 * CK, c * CK:(c + 1) * CK] = mid
            m = jnp.maximum(m, jnp.max(mid.reshape(CK // 8, 8, CK), axis=0))
        mb_s[u, b:b + 1, c * CK:(c + 1) * CK] = jnp.max(m, axis=0, keepdims=True)

    def b_values(h, i, u):
        b, c = i // PER, i % PER

        def vt(j):
            return vb_s[(j // PER) * H + h, :, (j % PER) * CK:(j % PER + 1) * CK]
        r0 = 2 * CK * b
        m = mb_s[u, b:b + 1, c * CK:(c + 1) * CK]
        pe = jnp.exp2(s_s[u, r0:r0 + CK, c * CK:(c + 1) * CK] - m)
        acc = _mm(vt(i), jnp.where(causal, pe, 0.0).astype(BF16))
        if i >= 1:
            pm = jnp.exp2(s_s[u, r0 + CK:r0 + 2 * CK, c * CK:(c + 1) * CK] - m)
            acc += _mm(vt(i - 1), pm.astype(BF16))
        if i >= 2:
            acc += _mm(vt(i - 2), jnp.where(causal, 0.0, pe).astype(BF16))
        o = acc * (1.0 / acc[DH:DH + 1, :])
        o_s[b, pl.ds(pl.multiple_of(h * HP, HP), HP), c * CK:(c + 1) * CK] = o.astype(BF16)

    def b_step(h, u, do_values, do_scores):
        for i in range(NC):
            if do_values:
                b_values(h, i, u)
            if do_scores:
                b_scores(h + UB if do_values else h, i, u)

    def b_attn():
        for u in range(UB):
            b_step(u, u, False, True)

        def body(i, _):
            for u in range(UB):
                b_step(i * UB + u, u, True, True)
            return _
        lax.fori_loop(0, H // UB - 1, body, None)
        for u in range(UB):
            b_step(H - UB + u, u, True, False)

    def b_out(b, _):
        x_s[b] = x_s[b] + _mm(wob_s[...], o_s[b])
        return _

    def layer_pair(r, _):
        with jax.named_scope("a_proj"):
            lax.fori_loop(0, NB, a_proj, None)
        with jax.named_scope("a_attn"):
            a_attn()
        with jax.named_scope("b_proj"):
            lax.fori_loop(0, NB, a_out_b_proj, None)
        with jax.named_scope("b_attn"):
            b_attn()
        with jax.named_scope("b_out"):
            lax.fori_loop(0, NB, b_out, None)
        return _
    lax.fori_loop(0, 2, layer_pair, None)

    for b in range(NB):
        out_ref[:, b * TB:(b + 1) * TB] = x_s[b].astype(BF16)


@jax.jit
def pallas_interleave_layers__grouped_kv_mqa__sliding_block__prompt_kernel(
        A_x, A_wq, A_wk, A_wv, A_wo, B_x, B_wqkv, B_wo):
    del B_x
    out_t = pl.pallas_call(
        _kernel,
        out_shape=jax.ShapeDtypeStruct((D, S), BF16),
        scratch_shapes=[
            pltpu.VMEM((NB, D, TB), F32),
            pltpu.VMEM((D + 2 * HP, D), BF16),
            pltpu.VMEM((D, H * HP), BF16),
            pltpu.VMEM((3 * D, D), BF16),
            pltpu.VMEM((D, H * HP), BF16),
            pltpu.VMEM((NB * H, HP, TB), BF16),
            pltpu.VMEM((S, HP), BF16),
            pltpu.VMEM((NB, HP, TB), BF16),
            pltpu.VMEM((NB, H * HP, TB), BF16),
            pltpu.VMEM((U, 8, TB), F32),
            pltpu.VMEM((U, S, TB), F32),
            pltpu.VMEM((H, S, HP), BF16),
            pltpu.VMEM((NB * H, HP, TB), BF16),
            pltpu.VMEM((UB, 8, TB), F32),
        ],
        compiler_params=pltpu.CompilerParams(vmem_limit_bytes=110 * 2**20),
    )(A_x.reshape(S, D).T, A_wq, A_wk.T, A_wv.T, A_wo, B_wqkv, B_wo)
    return out_t.T.reshape(1, S, D)
```

```python
import jax
import jax.numpy as jnp
import numpy as np
from jax import lax
import jax.experimental.pallas as pl
import jax.experimental.pallas.tpu as pltpu

S, D, H, DH, WIN = 2048, 448, 16, 28, 256
HP = 32
XR = 16
TB = 512
NB = S // TB
CK = 128
NC = S // CK
PER = TB // CK
MR = 64
UA = 4
UB = 4
NV = 208
VCH = [(j * NC + 8) // (NV // 16) for j in range(NV // 16)]
VROWS = [c * CK + CK - 16 + 8 * i for c in VCH for i in range(2)]
KB0 = max(UA, 2 * UB) * S
QSCALE = float(DH ** -0.5 * np.log2(np.e))
SUM_MIN, SUM_MAX = 2.0 ** -80, 2.0 * S
F32, BF16, U32 = jnp.float32, jnp.bfloat16, jnp.uint32


def _mm(a, b):
    return jnp.dot(a, b, preferred_element_type=F32)


def _merge(*streams):
    keyed = [((i + 0.5) / len(s), n, f) for n, s in enumerate(streams) for i, f in enumerate(s)]
    return [f for _, _, f in sorted(keyed, key=lambda e: e[:2])]


def _run(thunks):
    for f in thunks:
        f()


def _split_rows(v, parts):
    head = v.astype(BF16).astype(F32)
    row = lax.broadcasted_iota(jnp.int32, (XR, v.shape[1]), 0)
    out = jnp.zeros(row.shape, F32)
    for i, part in enumerate(parts):
        out = jnp.where(row == i, v - head if part else head, out)
    return out


def _with_column_sums(w):
    return jnp.concatenate([w, _split_rows(jnp.sum(w, axis=0, keepdims=True), (0, 1, 0))], axis=0)


def _key(b):
    return b if isinstance(b, int) else None


def _aligned(i, n):
    return i if isinstance(i, int) else pl.multiple_of(i, n)


def _kernel(xt_hbm, wq_hbm, wkt_hbm, wvt_hbm, wo_hbm, wqkv_hbm, bwo_hbm, out_hbm,
            h_s, wq_in, wkt_in, wvt_in, wo_in, wqkv_in, bwo_in, sems, zero_s,
            x_s, wa_s, woa_s, wb_s, wob_s, q_s, ka_s, va_s, o_s, mean_s, qn_s, kn_s, kv_s, unsafe_s,
            pa_s, pb_s, kb_s, kr_s, vb_s):
    def x_copy(b):
        return pltpu.make_async_copy(
            xt_hbm.at[:, pl.ds(_aligned(b * TB, TB), TB)], h_s.at[b, pl.ds(0, D)], sems.at[b])

    def out_copy(b):
        return pltpu.make_async_copy(
            h_s.at[b, pl.ds(0, D)], out_hbm.at[:, pl.ds(_aligned(b * TB, TB), TB)], sems.at[b])

    def last_out_copy(r):
        return pltpu.make_async_copy(
            h_s.at[NB - 1, pl.ds(r * MR, MR)], out_hbm.at[pl.ds(r * MR, MR), pl.ds(S - TB, TB)], sems.at[NB + r])

    wk_copy, wv_copy, wq_copy, *later_copies = [
        pltpu.make_async_copy(src, dst, sems.at[NB + D // MR + i]) for i, (src, dst) in enumerate(
            [(wkt_hbm, wkt_in), (wvt_hbm, wvt_in), (wq_hbm, wq_in),
             (wo_hbm, wo_in), (wqkv_hbm, wqkv_in), (bwo_hbm, bwo_in)])]

    ones_row = jnp.where(lax.broadcasted_iota(jnp.int32, (HP, TB), 0) == DH, 1.0, 0.0).astype(F32)
    spare = lax.broadcasted_iota(jnp.int32, (8, TB), 0) == DH % 8
    lane = lax.broadcasted_iota(jnp.int32, (HP, CK), 1)
    causal = lax.broadcasted_iota(jnp.int32, (CK, CK), 0) <= lax.broadcasted_iota(jnp.int32, (CK, CK), 1)
    scale, stats = {}, {}

    def moments(b, d, first):
        d = d.reshape(d.shape[0] // 8, 8, d.shape[1])
        s1, s2 = jnp.sum(d, axis=0), jnp.sum(d * d, axis=0)
        stats[_key(b)] = (s1, s2) if first else (stats[_key(b)][0] + s1, stats[_key(b)][1] + s2)

    def layernorm(b, first=False):
        def piece():
            s1, s2 = stats[_key(b)]
            mean = jnp.sum(s1, axis=0, keepdims=True) * (1.0 / D)
            var = jnp.sum(s2, axis=0, keepdims=True) * (1.0 / D) - mean * mean
            scale[_key(b)] = lax.rsqrt(jnp.maximum(var, 0.0) + 1e-5)
            h_s[b, D:, :] = _split_rows(-mean, (0, 0, 1)).astype(BF16)
            mean_s[b] = jnp.broadcast_to(mean, (8, TB)) if first else mean_s[b] + mean
        return [piece]

    def input_layernorm(b):
        return [lambda r=r: moments(b, h_s[b, r * MR:(r + 1) * MR, :].astype(F32), r == 0)
                for r in range(D // MR)] + layernorm(b, True)

    def per_head(w_s, r0, b, factor, emit):
        ys = []

        def piece(j):
            y = _mm(w_s[r0 + j * MR:r0 + (j + 1) * MR, :], h_s[b])
            ys.append(y * (scale[_key(b)] * factor if factor else scale[_key(b)]))
            for h in range(H):
                if j * MR < (h + 1) * DH <= (j + 1) * MR:
                    j0 = h * DH // MR
                    rows = jnp.concatenate(ys[j0:], axis=0)[h * DH - j0 * MR:(h + 1) * DH - j0 * MR]
                    emit(h, jnp.concatenate([rows, jnp.zeros((HP - DH, TB), F32)], axis=0))
        return [lambda j=j: piece(j) for j in range(D // MR)]

    def put_q(b):
        def emit(h, q):
            q_s[b * H + h] = q
            qn_s[b, h:h + 1, :] = jnp.sum(q * q, axis=0, keepdims=True)
        return emit

    def a_proj(b):
        def kv():
            y = _mm(wa_s[D:D + 2 * HP, :], h_s[b]) * scale[_key(b)]
            kn_s[b, 0:1, :] = jnp.sum(y[0:HP] * y[0:HP], axis=0, keepdims=True)
            k = (y[0:HP] + ones_row).T
            ka_s[pl.ds(_aligned(b * (TB // 2), TB // 2), TB // 2), :] = pltpu.bitcast(k.astype(BF16), U32)
            va_s[b] = pltpu.bitcast((y[HP:2 * HP] + ones_row).astype(BF16), U32)
            for g, k0 in enumerate(VROWS):
                if isinstance(b, int) and k0 // TB == b:
                    kv_s[8 * g:8 * g + 8, :] = k[k0 % TB:k0 % TB + 8]
        return [kv] + per_head(wa_s, 0, b, QSCALE, put_q(b))

    def b_proj(b):
        def put_k(h, k):
            kn_s[b, h:h + 1, :] = jnp.sum(k * k, axis=0, keepdims=True)
            k = k + ones_row
            for c in range(PER):
                kw = jnp.concatenate([k[:, c * CK:(c + 1) * CK]] * 4, axis=0).T
                parts = [jnp.where((lane >= g * HP) & (lane < (g + 1) * HP), kw[g * HP:(g + 1) * HP], 0.0)
                         for g in range(4)]
                t = b * PER + c
                kb_s[h, pl.ds(_aligned(t * CK, CK), CK), :] = jnp.concatenate(parts, axis=0).astype(BF16)
                kr_s[h, pl.ds(_aligned(t * HP, HP), HP), :] = (
                    (parts[0] + parts[1]) + (parts[2] + parts[3])).astype(BF16)

        def put_v(h, v):
            v = (v + ones_row).astype(BF16)
            for c in range(PER):
                vb_s[h, b * PER + c] = v[:, c * CK:(c + 1) * CK]
        return (per_head(wb_s, D, b, None, put_k) + per_head(wb_s, 0, b, QSCALE, put_q(b))
                + per_head(wb_s, 2 * D, b, None, put_v))

    def out_proj(w_s, b, first=False, last=False):
        def piece(r):
            rows = slice(r * MR, (r + 1) * MR)
            x = h_s[b, rows, :].astype(F32) if first else x_s[b, rows, :]
            x = x + _mm(w_s[rows, :], o_s[b])
            if last:
                h_s[b, rows, :] = x.astype(BF16)
            else:
                x_s[b, rows, :] = x
                d = (x.reshape(MR // 8, 8, TB) - mean_s[b]).reshape(MR, TB)
                h_s[b, rows, :] = d.astype(BF16)
                moments(b, d, r == 0)
        return [lambda r=r: piece(r) for r in range(D // MR)]

    def transposed(dst, src, pad_heads):
        def piece(c0, c1):
            w = src[:, c0:c1].astype(F32)
            if pad_heads:
                z = jnp.zeros((HP - DH, c1 - c0), F32)
                w = jnp.concatenate([p for h in range(H) for p in (w[h * DH:(h + 1) * DH], z)], axis=0)
            else:
                w = _with_column_sums(w)
            dst[c0:c1, :] = w.T.astype(BF16)
        n = src.shape[1]
        return [lambda c=c: piece(c, min(c + CK, n)) for c in range(0, n, CK)]

    def kv_weights():
        z = jnp.zeros((HP - DH, D), F32)
        w = jnp.concatenate([wkt_in[...].astype(F32), z, wvt_in[...].astype(F32), z], axis=0)
        wa_s[D:D + 2 * HP, :] = _with_column_sums(w.T).T.astype(BF16)

    def bound_scores(heads, order):
        k2 = jnp.max(jnp.max(kn_s[:, 0:heads, :], axis=0), axis=1, keepdims=True)
        shift = (-jnp.sqrt(qn_s[...] * k2)).astype(BF16).astype(F32)

        def piece(b, h):
            q_s[b * H + h, HP - 8:, :] = jnp.where(spare, shift[b, h:h + 1, :], q_s[b * H + h, HP - 8:, :])
        return [lambda b=b, h=h: piece(b, h) for b, h in order]

    def put_head(b, h, cols, o):
        o_s[b, pl.ds(_aligned(h * HP, HP), HP), cols] = o.astype(BF16)

    def finish(b, h, cols, acc):
        total = acc[HP - 8:]
        r = pl.reciprocal(total, approx=True)
        r = r * (2.0 - total * r)
        put_head(b, h, cols, acc * r[DH % 8:DH % 8 + 1])
        unsafe_s[:, cols] = jnp.where((total >= SUM_MIN) & (total <= SUM_MAX), unsafe_s[:, cols], 1.0)

    def key_slot(g, d):
        return KB0 + 8 * (g * DH + d)

    def spread_keys():
        def piece(g):
            k = kv_s[8 * g:8 * g + 8, :]
            for d in range(DH):
                pa_s[key_slot(g, d):key_slot(g, d) + 8, :] = jnp.broadcast_to(k[:, d:d + 1], (8, CK))
        return [lambda g=g: piece(g) for g in range(len(VROWS))]

    def put_weights(r0, p):
        pa_s[r0:r0 + p.shape[0], :] = p[:, :CK]
        pb_s[r0:r0 + p.shape[0], :] = p[:, CK:]

    def a_values(t, u):
        st = {}

        def piece(c):
            rows = slice(u * S + c * CK, u * S + (c + 1) * CK)
            v = pltpu.bitcast(va_s[c // PER, :, (c % PER) * CK:(c % PER + 1) * CK], BF16)
            d = _mm(v, jnp.concatenate([pa_s[rows, :], pb_s[rows, :]], axis=1).astype(BF16))
            st["acc"] = d if c == 0 else st["acc"] + d
            if c == NC - 1:
                finish(t // H, t % H, slice(None), st["acc"])
        return [lambda c=c: piece(c) for c in range(NC)]

    def a_weights(t, u, offload):
        st = {"stored": 0, "issued": 0}
        zero = zero_s[0]
        steps = [(j, half, d) for j in range(len(VCH)) for half in range(2) for d in range(DH)] if offload else []
        total = S - NV + 12 * NC

        def vector_scores(j, half, d):
            def row(i, c):
                return q_s[t, i:i + 1, c * CK:(c + 1) * CK]
            for g in (2 * j, 2 * j + 1):
                r = key_slot(g, d)
                k = pa_s[pl.ds(pl.multiple_of(zero + r, 8), 8) if d % 6 == 2 else slice(r, r + 8), :]
                for c in (2 * half, 2 * half + 1):
                    st[g, c] = (row(DH, c) if d == 0 else st[g, c]) + k * row(d, c)
                if d == DH - 1 and half == 1:
                    put_weights(u * S + VROWS[g], jnp.exp2(jnp.concatenate([st[g, c] for c in range(PER)], axis=1)))

        def piece(c):
            if c == 0:
                st["q"] = q_s[t].astype(BF16)
            k0, k1 = c * CK, (c + 1) * CK - (16 if offload and c in VCH else 0)
            s = _mm(pltpu.bitcast(ka_s[k0 // 2:k1 // 2, :], BF16), st["q"])
            for r0 in range(0, k1 - k0, 16):
                put_weights(u * S + k0 + r0, jnp.exp2(s[r0:r0 + 16]))
                st["stored"] += 16
                now = st["stored"] + 12 * (c + (r0 + 16 == k1 - k0)) + 24
                if u == UA - 1:
                    now = now * total // (total - 24)
                upto = min(-(-len(steps) * now // total), len(steps))
                for i in range(st["issued"], upto):
                    vector_scores(*steps[i])
                st["issued"] = upto
        return [lambda c=c: piece(c) for c in range(NC)]

    def a_block(base, n_values, n_weights, fill=()):
        values = [f for j in range(n_values) for f in a_values(base + j, j)]
        weights = [f for j in range(n_weights) for f in a_weights(base + n_values + j, j, n_values > 0)]
        _run(_merge(values, weights, list(fill)))

    def a_exact(t, _):
        q = q_s[t].astype(BF16)

        def scores(j):
            return _mm(pltpu.bitcast(ka_s[pl.ds(pl.multiple_of(j * (TB // 2), TB // 2), TB // 2), :], BF16), q)
        m = lax.fori_loop(0, NB, lambda j, m: jnp.maximum(m, jnp.max(scores(j), axis=0, keepdims=True)),
                          jnp.full((1, TB), -jnp.inf, F32))
        acc = lax.fori_loop(0, NB, lambda j, acc: acc + _mm(
            pltpu.bitcast(va_s[j], BF16), jnp.exp2(scores(j) - m).astype(BF16)), jnp.zeros((HP, TB), F32))
        put_head(t // H, t % H, slice(None), acc / acc[DH:DH + 1])
        return _

    def b_step(h0, u, do_values, do_weights):
        st = {}

        def by_group(right, left):
            parts = [right[0:HP]]
            for g in range(1, 4):
                rows = slice(g * HP, (g + 1) * HP)
                parts.append(jnp.where(lane >= g * HP, right[rows], left[rows]))
            return jnp.concatenate(parts, axis=0)

        def weights(i):
            h = h0 + UB if do_values else h0
            q0, q1 = (q_s[j // PER * H + h, :, j % PER * CK:(j % PER + 1) * CK] for j in (i, min(i + 1, NC - 1)))
            w = jnp.concatenate([q0] + [jnp.where(lane >= g * HP, q0, q1) for g in range(1, 4)], axis=0).astype(BF16)
            before = _mm(kb_s[h, (i - 1) * CK:i * CK, :], w) if i >= 1 else None
            same = _mm(kb_s[h, i * CK:(i + 1) * CK, :], w)
            if i >= 2:
                wr = jnp.concatenate([jnp.where((lane >= g * HP) & (lane < (g + 1) * HP), q0, 0.0)
                                      for g in range(4)], axis=0)
                r = _mm(kr_s[h, (i - 2) * HP:(i - 1) * HP, :], wr.astype(BF16))
                oldest = by_group(jnp.concatenate([r] * 4, axis=0), st["before"])
            else:
                oldest = -jnp.inf
            r0 = (u * NC + i) * 2 * CK
            pa_s[r0:r0 + CK, :] = jnp.exp2(jnp.where(causal, same, oldest))
            if i >= 1:
                pa_s[r0 + CK:r0 + 2 * CK, :] = jnp.exp2(by_group(before, st["same"]))
            st["same"], st["before"] = same, before

        def values(i):
            r0 = (u * NC + i) * 2 * CK
            edge = pa_s[r0:r0 + CK, :]
            acc = _mm(vb_s[h0, i], jnp.where(causal, edge, 0.0).astype(BF16))
            if i >= 1:
                acc += _mm(vb_s[h0, i - 1], pa_s[r0 + CK:r0 + 2 * CK, :].astype(BF16))
            if i >= 2:
                acc += _mm(vb_s[h0, i - 2], jnp.where(causal, 0.0, edge).astype(BF16))
            finish(i // PER, h0, slice(i % PER * CK, (i % PER + 1) * CK), acc)
        fs = ([values] if do_values else []) + ([weights] if do_weights else [])
        return [lambda f=f, i=i: f(i) for i in range(NC) for f in fs]

    def b_exact(t, _):
        b, h = t // H, t % H
        for c in range(PER):
            cols = slice(c * CK, (c + 1) * CK)
            j0 = jnp.maximum(b * PER + c - 2, 0)
            s = _mm(kb_s[h, pl.ds(pl.multiple_of(j0 * CK, CK), 3 * CK), :],
                    jnp.concatenate([q_s[t, :, cols]] * 4, axis=0).astype(BF16))
            age = ((b * PER + c - j0) * CK + lax.broadcasted_iota(jnp.int32, s.shape, 1)
                   - lax.broadcasted_iota(jnp.int32, s.shape, 0))
            s = jnp.where((age >= 0) & (age < WIN), s, -jnp.inf)
            p = jnp.exp2(s - jnp.max(s, axis=0, keepdims=True)).astype(BF16)
            acc = sum(_mm(vb_s[h, j0 + j], p[j * CK:(j + 1) * CK]) for j in range(3))
            put_head(b, h, cols, acc / acc[DH:DH + 1])
        return _

    zero_s[0] = 0
    unsafe_s[...] = jnp.zeros(unsafe_s.shape, F32)

    for cp in [wk_copy, wv_copy, x_copy(0), wq_copy] + [x_copy(b) for b in range(1, NB)] + later_copies:
        cp.start()
    wq_t, p0, p1 = transposed(wa_s, wq_in, False), a_proj(0), a_proj(1)
    wk_copy.wait()
    wv_copy.wait()
    kv_weights()
    x_copy(0).wait()
    _run(input_layernorm(0) + p0[:1])
    wq_copy.wait()
    _run([wq_t[0], wq_t[1], p0[1], wq_t[2], p0[2], wq_t[3]])
    x_copy(1).wait()
    _run(_merge(p0[3:], input_layernorm(1)) + p1[:3])
    x_copy(2).wait()
    x_copy(3).wait()
    _run(_merge(p1[3:], input_layernorm(2)))
    _run(_merge(a_proj(2), input_layernorm(3)))
    _run(a_proj(3))

    for first in (True, False):
        bounds = bound_scores(1, [divmod(t, H) for t in range(NB * H)])
        _run(bounds[:UA])
        a_block(0, 0, UA, _merge(bounds[UA:], spread_keys()))
        if first:
            for cp in later_copies:
                cp.wait()
        lax.fori_loop(0, NB * H // UA - 1, lambda i, _: a_block(i * UA, UA, UA), None)
        a_block(NB * H - UA, UA, 0, transposed(woa_s, wo_in, True) if first else ())

        out = [out_proj(woa_s, b, first=first) + layernorm(b) for b in range(NB)]
        _run(_merge(out[0] + out[1], transposed(wb_s, wqkv_in, False) if first else []))
        _run(b_proj(0) + out[2] + b_proj(1) + out[3] + b_proj(2))
        _run(_merge(b_proj(3), transposed(wob_s, bwo_in, True) if first else []))

        bounds = bound_scores(H, [(b, h) for h in range(H) for b in range(NB)])
        _run(bounds[:NB])
        _run(_merge([f for u in range(UB) for f in b_step(u, u, False, True)], bounds[NB:]))
        lax.fori_loop(0, H // UB - 1,
                      lambda i, _: _run([f for u in range(UB) for f in b_step(i * UB + u, u, True, True)]), None)
        _run([f for u in range(UB) for f in b_step(H - UB + u, u, True, False)])

        if first:
            out = [out_proj(wob_s, b) + layernorm(b) for b in range(NB)]
            _run(out[0] + out[1] + a_proj(0) + out[2] + a_proj(1) + out[3] + a_proj(2) + a_proj(3))

    for b in range(NB - 1):
        _run(out_proj(wob_s, b, last=True))
        out_copy(b).start()
    for r, f in enumerate(out_proj(wob_s, NB - 1, last=True)):
        f()
        last_out_copy(r).start()
    unsafe = jnp.max(jnp.where(spare, unsafe_s[...], 0.0)) > 0.0
    for b in range(NB - 1):
        out_copy(b).wait()
    for r in range(D // MR):
        last_out_copy(r).wait()

    @pl.when(unsafe)
    def _():
        def blocks(stages):
            lax.fori_loop(0, NB, lambda b, _: _run(stages(b)), None)

        def reload(b):
            x_copy(b).start()
            x_copy(b).wait()
            x_s[b] = h_s[b, 0:D, :].astype(F32)
            return input_layernorm(b) + a_proj(b)

        def layer_pair(r, _):
            lax.fori_loop(0, NB * H, a_exact, None)
            blocks(lambda b: out_proj(woa_s, b) + layernorm(b) + b_proj(b))
            lax.fori_loop(0, NB * H, b_exact, None)
            blocks(lambda b: out_proj(wob_s, b) + layernorm(b) + a_proj(b))

        def store(b, _):
            h_s[b, 0:D, :] = x_s[b].astype(BF16)
            out_copy(b).start()
            out_copy(b).wait()
        blocks(reload)
        lax.fori_loop(0, 2, layer_pair, None)
        lax.fori_loop(0, NB, store, None)


@jax.jit
def pallas_interleave_layers__grouped_kv_mqa__sliding_block__prompt_kernel(
    A_x: jax.Array,
    A_wq: jax.Array,
    A_wk: jax.Array,
    A_wv: jax.Array,
    A_wo: jax.Array,
    B_x: jax.Array,
    B_wqkv: jax.Array,
    B_wo: jax.Array,
):
    del B_x
    out_t = pl.pallas_call(
        _kernel,
        out_shape=jax.ShapeDtypeStruct((D, S), BF16),
        in_specs=[pl.BlockSpec(memory_space=pl.ANY)] * 7,
        out_specs=pl.BlockSpec(memory_space=pl.ANY),
        scratch_shapes=[
            pltpu.VMEM((NB, D + XR, TB), BF16),
            pltpu.VMEM((D, D), BF16),
            pltpu.VMEM((DH, D), BF16),
            pltpu.VMEM((DH, D), BF16),
            pltpu.VMEM((D, D), BF16),
            pltpu.VMEM((D, 3 * D), BF16),
            pltpu.VMEM((D, D), BF16),
            pltpu.SemaphoreType.DMA((NB + D // MR + 6,)),
            pltpu.SMEM((1,), jnp.int32),
            pltpu.VMEM((NB, D, TB), F32),
            pltpu.VMEM((D + 2 * HP, D + XR), BF16),
            pltpu.VMEM((D, H * HP), BF16),
            pltpu.VMEM((3 * D, D + XR), BF16),
            pltpu.VMEM((D, H * HP), BF16),
            pltpu.VMEM((NB * H, HP, TB), F32),
            pltpu.VMEM((S // 2, HP), U32),
            pltpu.VMEM((NB, HP // 2, TB), U32),
            pltpu.VMEM((NB, H * HP, TB), BF16),
            pltpu.VMEM((NB, 8, TB), F32),
            pltpu.VMEM((NB, H, TB), F32),
            pltpu.VMEM((NB, H, TB), F32),
            pltpu.VMEM((2 * CK, HP), F32),
            pltpu.VMEM((8, TB), F32),
            pltpu.VMEM((KB0 + NV * DH, CK), F32),
            pltpu.VMEM((UA * S, TB - CK), F32),
            pltpu.VMEM((H, S, CK), BF16),
            pltpu.VMEM((H, NC * HP, CK), BF16),
            pltpu.VMEM((H, NC, HP, CK), BF16),
        ],
        compiler_params=pltpu.CompilerParams(vmem_limit_bytes=100 * 2**20),
    )(A_x.reshape(S, D).T, A_wq, A_wk.T, A_wv.T, A_wo, B_wqkv, B_wo)
    return out_t.T.reshape(1, S, D)
```

```python
import jax
import jax.numpy as jnp
import numpy as np
from jax import lax
import jax.experimental.pallas as pl
import jax.experimental.pallas.tpu as pltpu

S, D, H, DH, WIN = 2048, 448, 16, 28, 256
HP = 32
HD = DH // 2
XR = 16
TB = 512
NB = S // TB
CK = 128
NC = S // CK
PER = TB // CK
MR = 64
UA = 4
UB = 4
VK = 16
LEAD = 26
KB0 = max(UA, 2 * UB) * S
assert LEAD < 6 * HD
QSCALE = float(DH ** -0.5 * np.log2(np.e))
SUM_MIN, SUM_MAX = 2.0 ** -80, 2.0 * S
F32, BF16, U32 = jnp.float32, jnp.bfloat16, jnp.uint32


def _mm(a, b):
    return jnp.dot(a, b, preferred_element_type=F32)


def _merge(*streams):
    keyed = [((i + 0.5) / len(s), n, f) for n, s in enumerate(streams) for i, f in enumerate(s)]
    return [f for _, _, f in sorted(keyed, key=lambda e: e[:2])]


def _run(thunks):
    for f in thunks:
        f()


def _split_rows(v, parts):
    head = v.astype(BF16).astype(F32)
    row = lax.broadcasted_iota(jnp.int32, (XR, v.shape[1]), 0)
    out = jnp.zeros(row.shape, F32)
    for i, part in enumerate(parts):
        out = jnp.where(row == i, v - head if part else head, out)
    return out


def _with_column_sums(w):
    return jnp.concatenate([w, _split_rows(jnp.sum(w, axis=0, keepdims=True), (0, 1, 0))], axis=0)


def _key(b):
    return b if isinstance(b, int) else None


def _aligned(i, n):
    return i if isinstance(i, int) else pl.multiple_of(i, n)


def _kernel(xt_hbm, wq_hbm, wkt_hbm, wvt_hbm, wo_hbm, wqkv_hbm, bwo_hbm, out_hbm,
            h_s, wq_in, wkt_in, wvt_in, wo_in, wqkv_in, bwo_in, sems, zero_s,
            x_s, wa_s, woa_s, wb_s, wob_s, q_s, qf_s, ka_s, va_s, o_s, mean_s, qn_s, kn_s, kv_s, unsafe_s,
            pa_s, pb_s, kb_s, kr_s, vb_s):
    def x_copy(b):
        return pltpu.make_async_copy(
            xt_hbm.at[:, pl.ds(_aligned(b * TB, TB), TB)], h_s.at[b, pl.ds(0, D)], sems.at[b])

    def out_copy(b):
        return pltpu.make_async_copy(
            h_s.at[b, pl.ds(0, D)], out_hbm.at[:, pl.ds(_aligned(b * TB, TB), TB)], sems.at[b])

    def last_out_copy(r):
        return pltpu.make_async_copy(
            h_s.at[NB - 1, pl.ds(r * MR, MR)], out_hbm.at[pl.ds(r * MR, MR), pl.ds(S - TB, TB)], sems.at[NB + r])

    wk_copy, wv_copy, wq_copy, *later_copies = [
        pltpu.make_async_copy(src, dst, sems.at[NB + D // MR + i]) for i, (src, dst) in enumerate(
            [(wkt_hbm, wkt_in), (wvt_hbm, wvt_in), (wq_hbm, wq_in),
             (wo_hbm, wo_in), (wqkv_hbm, wqkv_in), (bwo_hbm, bwo_in)])]

    ones_row = jnp.where(lax.broadcasted_iota(jnp.int32, (HP, TB), 0) == DH, 1.0, 0.0).astype(F32)
    spare = lax.broadcasted_iota(jnp.int32, (8, TB), 0) == DH % 8
    lane = lax.broadcasted_iota(jnp.int32, (HP, CK), 1)
    causal = lax.broadcasted_iota(jnp.int32, (CK, CK), 0) <= lax.broadcasted_iota(jnp.int32, (CK, CK), 1)
    scale, stats = {}, {}

    def moments(b, d, first):
        d = d.reshape(d.shape[0] // 8, 8, d.shape[1])
        s1, s2 = jnp.sum(d, axis=0), jnp.sum(d * d, axis=0)
        stats[_key(b)] = (s1, s2) if first else (stats[_key(b)][0] + s1, stats[_key(b)][1] + s2)

    def layernorm(b, first=False):
        def piece():
            s1, s2 = stats[_key(b)]
            mean = jnp.sum(s1, axis=0, keepdims=True) * (1.0 / D)
            var = jnp.sum(s2, axis=0, keepdims=True) * (1.0 / D) - mean * mean
            scale[_key(b)] = lax.rsqrt(jnp.maximum(var, 0.0) + 1e-5)
            h_s[b, D:, :] = _split_rows(-mean, (0, 0, 1)).astype(BF16)
            mean_s[b] = jnp.broadcast_to(mean, (8, TB)) if first else mean_s[b] + mean
        return [piece]

    def input_layernorm(b):
        return [lambda r=r: moments(b, h_s[b, r * MR:(r + 1) * MR, :].astype(F32), r == 0)
                for r in range(D // MR)] + layernorm(b, True)

    def per_head(w_s, r0, b, factor, emit):
        ys = []

        def piece(j):
            y = _mm(w_s[r0 + j * MR:r0 + (j + 1) * MR, :], h_s[b])
            ys.append(y * (scale[_key(b)] * factor if factor else scale[_key(b)]))
            for h in range(H):
                if j * MR < (h + 1) * DH <= (j + 1) * MR:
                    j0 = h * DH // MR
                    rows = jnp.concatenate(ys[j0:], axis=0)[h * DH - j0 * MR:(h + 1) * DH - j0 * MR]
                    emit(h, jnp.concatenate([rows, jnp.zeros((HP - DH, TB), F32)], axis=0))
        return [lambda j=j: piece(j) for j in range(D // MR)]

    def put_q(b, factors=False):
        def emit(h, q):
            q_s[b * H + h] = q
            if factors:
                b11, b12, b21, b22 = (jnp.concatenate([x[:, c * CK:(c + 1) * CK] for c in (i, i + 2)], axis=1)
                                      for x in (q[0:16], q[HD:HD + 16]) for i in (0, 1))
                qf_s[b * H + h] = jnp.concatenate([b21 - b11, b11 + b22, b21 + b22, b12 - b22, b11 + b12], axis=0)
            qn_s[b, h:h + 1, :] = jnp.sum(q * q, axis=0, keepdims=True)
        return emit

    def a_proj(b):
        def kv():
            y = _mm(wa_s[D:D + 2 * HP, :], h_s[b]) * scale[_key(b)]
            kn_s[b, 0:1, :] = jnp.sum(y[0:HP] * y[0:HP], axis=0, keepdims=True)
            k = (y[0:HP] + ones_row).T
            ka_s[pl.ds(_aligned(b * (TB // 2), TB // 2), TB // 2), :] = pltpu.bitcast(k.astype(BF16), U32)
            va_s[b] = pltpu.bitcast((y[HP:2 * HP] + ones_row).astype(BF16), U32)
            for c in range(PER):
                kv_s[pl.ds(_aligned((b * PER + c) * VK, VK), VK), :] = k[(c + 1) * CK - VK:(c + 1) * CK]
        return [kv] + per_head(wa_s, 0, b, QSCALE, put_q(b, True))

    def b_proj(b):
        def put_k(h, k):
            kn_s[b, h:h + 1, :] = jnp.sum(k * k, axis=0, keepdims=True)
            k = k + ones_row
            for c in range(PER):
                kw = jnp.concatenate([k[:, c * CK:(c + 1) * CK]] * 4, axis=0).T
                parts = [jnp.where((lane >= g * HP) & (lane < (g + 1) * HP), kw[g * HP:(g + 1) * HP], 0.0)
                         for g in range(4)]
                t = b * PER + c
                kb_s[h, pl.ds(_aligned(t * CK, CK), CK), :] = jnp.concatenate(parts, axis=0).astype(BF16)
                kr_s[h, pl.ds(_aligned(t * HP, HP), HP), :] = (
                    (parts[0] + parts[1]) + (parts[2] + parts[3])).astype(BF16)

        def put_v(h, v):
            v = (v + ones_row).astype(BF16)
            for c in range(PER):
                vb_s[h, b * PER + c] = v[:, c * CK:(c + 1) * CK]
        return _merge(per_head(wb_s, D, b, None, put_k),
                      per_head(wb_s, 0, b, QSCALE, put_q(b)) + per_head(wb_s, 2 * D, b, None, put_v))

    def out_proj(w_s, b, first=False, last=False):
        def piece(r):
            rows = slice(r * MR, (r + 1) * MR)
            x = h_s[b, rows, :].astype(F32) if first else x_s[b, rows, :]
            x = x + _mm(w_s[rows, :], o_s[b])
            if last:
                h_s[b, rows, :] = x.astype(BF16)
            else:
                x_s[b, rows, :] = x
                d = (x.reshape(MR // 8, 8, TB) - mean_s[b]).reshape(MR, TB)
                h_s[b, rows, :] = d.astype(BF16)
                moments(b, d, r == 0)
        return [lambda r=r: piece(r) for r in range(D // MR)]

    def transposed(dst, src, pad_heads):
        def piece(c0, c1):
            w = src[:, c0:c1].astype(F32)
            if pad_heads:
                z = jnp.zeros((HP - DH, c1 - c0), F32)
                w = jnp.concatenate([p for h in range(H) for p in (w[h * DH:(h + 1) * DH], z)], axis=0)
            else:
                w = _with_column_sums(w)
            dst[c0:c1, :] = w.T.astype(BF16)
        n = src.shape[1]
        return [lambda c=c: piece(c, min(c + CK, n)) for c in range(0, n, CK)]

    def kv_weights():
        z = jnp.zeros((HP - DH, D), F32)
        w = jnp.concatenate([wkt_in[...].astype(F32), z, wvt_in[...].astype(F32), z], axis=0)
        wa_s[D:D + 2 * HP, :] = _with_column_sums(w.T).T.astype(BF16)

    def bound_scores(heads, order):
        k2 = jnp.max(jnp.max(kn_s[:, 0:heads, :], axis=0), axis=1, keepdims=True)
        shift = (-jnp.sqrt(qn_s[...] * k2)).astype(BF16).astype(F32)

        def piece(b, h):
            q_s[b * H + h, HP - 8:, :] = jnp.where(spare, shift[b, h:h + 1, :], q_s[b * H + h, HP - 8:, :])
        return [lambda b=b, h=h: piece(b, h) for b, h in order]

    def put_head(b, h, cols, o):
        o_s[b, pl.ds(_aligned(h * HP, HP), HP), cols] = o.astype(BF16)

    def finish(b, h, cols, acc):
        total = acc[HP - 8:]
        r = pl.reciprocal(total, approx=True)
        r = r * (2.0 - total * r)
        put_head(b, h, cols, acc * r[DH % 8:DH % 8 + 1])
        unsafe_s[:, cols] = jnp.where((total >= SUM_MIN) & (total <= SUM_MAX), unsafe_s[:, cols], 1.0)

    def key_rows(j, m, d, zero):
        r = KB0 + 8 * ((j * 7 + m) * HD + d)
        return slice(r, r + 8) if zero is None else pl.ds(pl.multiple_of(zero + r, 8), 8)

    def spread_keys():
        def piece(j, d):
            a11, a12, a21, a22 = (jnp.broadcast_to(kv_s[VK * j + r:VK * j + r + 8, i:i + 1], (8, CK))
                                  for r in (0, 8) for i in (d, HD + d))
            for m, a in enumerate((a22, a21 + a22, a11 + a22, a12 - a22, a11 + a12, a11, a21 - a11)):
                pa_s[key_rows(j, m, d, zero_s[0] if m == 0 else None), :] = a
        return [lambda j=j, d=d: piece(j, d) for j in range(NC) for d in range(HD)]

    def put_weights(r0, p):
        pa_s[r0:r0 + p.shape[0], :] = p[:, :CK]
        pb_s[r0:r0 + p.shape[0], :] = p[:, CK:]

    def a_values(t, u):
        st = {}

        def piece(c):
            rows = slice(u * S + c * CK, u * S + (c + 1) * CK)
            v = pltpu.bitcast(va_s[c // PER, :, (c % PER) * CK:(c % PER + 1) * CK], BF16)
            d = _mm(v, jnp.concatenate([pa_s[rows, :], pb_s[rows, :]], axis=1).astype(BF16))
            st["acc"] = d if c == 0 else st["acc"] + d
            if c == NC - 1:
                finish(t // H, t % H, slice(None), st["acc"])
        return [lambda c=c: piece(c) for c in range(NC)]

    def vector_scores(t, u):
        st = {}
        zero = zero_s[0]

        def piece(j, m, d, tied):
            k = pa_s[key_rows(j, m, d, zero if tied else None), :]
            for half in range(2):
                left, right = (slice(c * CK, (c + 1) * CK) for c in (2 * half, 2 * half + 1))
                if m == 1:
                    q = q_s[t, d:d + 1, left]
                elif m == 4:
                    q = q_s[t, HD + d:HD + d + 1, right]
                else:
                    i = 16 * (m - (m > 1) - (m > 4)) + d
                    q = qf_s[t, i:i + 1, half * CK:(half + 1) * CK]
                if d > 0:
                    st[half] = st[half] + k * q
                elif m in (0, 5):
                    st[half] = q_s[t, DH:DH + 1, left if m == 0 else right] + k * q
                else:
                    st[half] = k * q
                if d == HD - 1:
                    p, c = st[half], st.setdefault((j, half), {})
                    if m == 0:
                        c[11] = p
                    elif m == 1:
                        c[21], c[22] = c[11] + p, p
                    elif m == 2:
                        c[11], c[22] = c[11] + p, p - c[22]
                    elif m == 3:
                        c[11] = c[11] + p
                    elif m == 4:
                        c[11], c[12] = c[11] - p, p
                    elif m == 5:
                        c[12], c[22] = c[12] + p, c[22] + p
                    else:
                        c[22] = c[22] + p
            if d == HD - 1 and m >= 5:
                g = m - 5
                s = [st[j, half][10 * g + c] for half in range(2) for c in (11, 12)]
                put_weights(u * S + (j + 1) * CK - VK + 8 * g, jnp.exp2(jnp.concatenate(s, axis=1)))
        return [lambda tied, j=j, m=m, d=d: piece(j, m, d, tied)
                for j in range(NC) for m in range(7) for d in range(HD)]

    def a_weights(t, u, tick=None):
        st = {}

        def piece(c):
            if c == 0:
                st["q"] = q_s[t].astype(BF16)
            k0, k1 = c * CK, (c + 1) * CK - (VK if tick else 0)
            s = _mm(pltpu.bitcast(ka_s[k0 // 2:k1 // 2, :], BF16), st["q"])
            for r0 in range(k0, k1, 16):
                put_weights(u * S + r0, jnp.exp2(s[r0 - k0:r0 - k0 + 16]))
                if tick:
                    tick((r0 - k0) // 16)
        return [lambda c=c: piece(c) for c in range(NC)]

    def a_block(base, n_values, n_weights, fill=()):
        tick = None
        if n_values and n_weights:
            steps = [f for j in range(n_weights) for f in vector_scores(base + n_values + j, j)]
            lead = [LEAD]

            def tick(i):
                n = lead[0] + (12 if i < 6 else 7 * HD - 6 * 12)
                for x, f in enumerate(steps[:n]):
                    y = x - lead[0]
                    f(y == 0 or (i == 6 and y == 8) or (y < 0 and x % 12 == 0))
                del steps[:n]
                lead[0] = 0
        values = [f for j in range(n_values) for f in a_values(base + j, j)]
        weights = [f for j in range(n_weights) for f in a_weights(base + n_values + j, j, tick)]
        _run(_merge(values, weights, list(fill)))

    def a_exact(t, _):
        q = q_s[t].astype(BF16)

        def scores(j):
            return _mm(pltpu.bitcast(ka_s[pl.ds(pl.multiple_of(j * (TB // 2), TB // 2), TB // 2), :], BF16), q)
        m = lax.fori_loop(0, NB, lambda j, m: jnp.maximum(m, jnp.max(scores(j), axis=0, keepdims=True)),
                          jnp.full((1, TB), -jnp.inf, F32))
        acc = lax.fori_loop(0, NB, lambda j, acc: acc + _mm(
            pltpu.bitcast(va_s[j], BF16), jnp.exp2(scores(j) - m).astype(BF16)), jnp.zeros((HP, TB), F32))
        put_head(t // H, t % H, slice(None), acc / acc[DH:DH + 1])
        return _

    def b_step(h0, u, do_values, do_weights):
        st = {}

        def by_group(right, left):
            parts = [right[0:HP]]
            for g in range(1, 4):
                rows = slice(g * HP, (g + 1) * HP)
                parts.append(jnp.where(lane >= g * HP, right[rows], left[rows]))
            return jnp.concatenate(parts, axis=0)

        def weights(i):
            h = h0 + UB if do_values else h0
            q0, q1 = (q_s[j // PER * H + h, :, j % PER * CK:(j % PER + 1) * CK] for j in (i, min(i + 1, NC - 1)))
            w = jnp.concatenate([q0] + [jnp.where(lane >= g * HP, q0, q1) for g in range(1, 4)], axis=0).astype(BF16)
            before = _mm(kb_s[h, (i - 1) * CK:i * CK, :], w) if i >= 1 else None
            same = _mm(kb_s[h, i * CK:(i + 1) * CK, :], w)
            if i >= 2:
                wr = jnp.concatenate([jnp.where((lane >= g * HP) & (lane < (g + 1) * HP), q0, 0.0)
                                      for g in range(4)], axis=0)
                r = _mm(kr_s[h, (i - 2) * HP:(i - 1) * HP, :], wr.astype(BF16))
                oldest = by_group(jnp.concatenate([r] * 4, axis=0), st["before"])
            else:
                oldest = -jnp.inf
            r0 = (u * NC + i) * 2 * CK
            pa_s[r0:r0 + CK, :] = jnp.exp2(jnp.where(causal, same, oldest))
            if i >= 1:
                pa_s[r0 + CK:r0 + 2 * CK, :] = jnp.exp2(by_group(before, st["same"]))
            st["same"], st["before"] = same, before

        def values(i):
            r0 = (u * NC + i) * 2 * CK
            edge = pa_s[r0:r0 + CK, :]
            acc = _mm(vb_s[h0, i], jnp.where(causal, edge, 0.0).astype(BF16))
            if i >= 1:
                acc += _mm(vb_s[h0, i - 1], pa_s[r0 + CK:r0 + 2 * CK, :].astype(BF16))
            if i >= 2:
                acc += _mm(vb_s[h0, i - 2], jnp.where(causal, 0.0, edge).astype(BF16))
            finish(i // PER, h0, slice(i % PER * CK, (i % PER + 1) * CK), acc)
        fs = ([values] if do_values else []) + ([weights] if do_weights else [])
        return [lambda f=f, i=i: f(i) for i in range(NC) for f in fs]

    def b_exact(t, _):
        b, h = t // H, t % H
        for c in range(PER):
            cols = slice(c * CK, (c + 1) * CK)
            j0 = jnp.maximum(b * PER + c - 2, 0)
            s = _mm(kb_s[h, pl.ds(pl.multiple_of(j0 * CK, CK), 3 * CK), :],
                    jnp.concatenate([q_s[t, :, cols]] * 4, axis=0).astype(BF16))
            age = ((b * PER + c - j0) * CK + lax.broadcasted_iota(jnp.int32, s.shape, 1)
                   - lax.broadcasted_iota(jnp.int32, s.shape, 0))
            s = jnp.where((age >= 0) & (age < WIN), s, -jnp.inf)
            p = jnp.exp2(s - jnp.max(s, axis=0, keepdims=True)).astype(BF16)
            acc = sum(_mm(vb_s[h, j0 + j], p[j * CK:(j + 1) * CK]) for j in range(3))
            put_head(b, h, cols, acc / acc[DH:DH + 1])
        return _

    zero_s[0] = 0
    unsafe_s[...] = jnp.zeros(unsafe_s.shape, F32)

    for cp in [wk_copy, wv_copy, x_copy(0), wq_copy] + [x_copy(b) for b in range(1, NB)] + later_copies:
        cp.start()
    wq_t, p0, p1 = transposed(wa_s, wq_in, False), a_proj(0), a_proj(1)
    wk_copy.wait()
    wv_copy.wait()
    kv_weights()
    x_copy(0).wait()
    _run(input_layernorm(0) + p0[:1])
    wq_copy.wait()
    _run([wq_t[0], wq_t[1], p0[1], wq_t[2], p0[2], wq_t[3]])
    x_copy(1).wait()
    _run(_merge(p0[3:], input_layernorm(1)) + p1[:3])
    x_copy(2).wait()
    x_copy(3).wait()
    _run(_merge(p1[3:], input_layernorm(2)))
    _run(_merge(a_proj(2), input_layernorm(3)))
    _run(a_proj(3))

    for first in (True, False):
        bounds = bound_scores(1, [divmod(t, H) for t in range(NB * H)])
        _run(bounds[:UA])
        a_block(0, 0, UA, _merge(bounds[UA:], spread_keys()))
        if first:
            for cp in later_copies:
                cp.wait()
        lax.fori_loop(0, NB * H // UA - 1, lambda i, _: a_block(i * UA, UA, UA), None)
        a_block(NB * H - UA, UA, 0, transposed(woa_s, wo_in, True) if first else ())

        out = [f for b in range(NB) for f in out_proj(woa_s, b, first=first) + layernorm(b)]
        _run(_merge(out, transposed(wb_s, wqkv_in, False) if first else []))
        _run(b_proj(0) + b_proj(1) + b_proj(2))
        _run(_merge(b_proj(3), transposed(wob_s, bwo_in, True) if first else []))

        bounds = bound_scores(H, [(b, h) for h in range(H) for b in range(NB)])
        _run(bounds[:NB])
        _run(_merge([f for u in range(UB) for f in b_step(u, u, False, True)], bounds[NB:]))
        lax.fori_loop(0, H // UB - 1,
                      lambda i, _: _run([f for u in range(UB) for f in b_step(i * UB + u, u, True, True)]), None)
        _run([f for u in range(UB) for f in b_step(H - UB + u, u, True, False)])

        if first:
            _run([f for b in range(NB) for f in out_proj(wob_s, b) + layernorm(b)])
            _run([f for b in range(NB) for f in a_proj(b)])

    for b in range(NB - 1):
        _run(out_proj(wob_s, b, last=True))
        out_copy(b).start()
    for r, f in enumerate(out_proj(wob_s, NB - 1, last=True)):
        f()
        last_out_copy(r).start()
    unsafe = jnp.max(jnp.where(spare, unsafe_s[...], 0.0)) > 0.0
    for b in range(NB - 1):
        out_copy(b).wait()
    for r in range(D // MR):
        last_out_copy(r).wait()

    @pl.when(unsafe)
    def _():
        def blocks(stages):
            lax.fori_loop(0, NB, lambda b, _: _run(stages(b)), None)

        def reload(b):
            x_copy(b).start()
            x_copy(b).wait()
            x_s[b] = h_s[b, 0:D, :].astype(F32)
            return input_layernorm(b) + a_proj(b)

        def layer_pair(r, _):
            lax.fori_loop(0, NB * H, a_exact, None)
            blocks(lambda b: out_proj(woa_s, b) + layernorm(b) + b_proj(b))
            lax.fori_loop(0, NB * H, b_exact, None)
            blocks(lambda b: out_proj(wob_s, b) + layernorm(b) + a_proj(b))

        def store(b, _):
            h_s[b, 0:D, :] = x_s[b].astype(BF16)
            out_copy(b).start()
            out_copy(b).wait()
        blocks(reload)
        lax.fori_loop(0, 2, layer_pair, None)
        lax.fori_loop(0, NB, store, None)


@jax.jit
def pallas_interleave_layers__grouped_kv_mqa__sliding_block__prompt_kernel(
    A_x: jax.Array,
    A_wq: jax.Array,
    A_wk: jax.Array,
    A_wv: jax.Array,
    A_wo: jax.Array,
    B_x: jax.Array,
    B_wqkv: jax.Array,
    B_wo: jax.Array,
):
    del B_x
    out_t = pl.pallas_call(
        _kernel,
        out_shape=jax.ShapeDtypeStruct((D, S), BF16),
        in_specs=[pl.BlockSpec(memory_space=pl.ANY)] * 7,
        out_specs=pl.BlockSpec(memory_space=pl.ANY),
        scratch_shapes=[
            pltpu.VMEM((NB, D + XR, TB), BF16),
            pltpu.VMEM((D, D), BF16),
            pltpu.VMEM((DH, D), BF16),
            pltpu.VMEM((DH, D), BF16),
            pltpu.VMEM((D, D), BF16),
            pltpu.VMEM((D, 3 * D), BF16),
            pltpu.VMEM((D, D), BF16),
            pltpu.SemaphoreType.DMA((NB + D // MR + 6,)),
            pltpu.SMEM((1,), jnp.int32),
            pltpu.VMEM((NB, D, TB), F32),
            pltpu.VMEM((D + 2 * HP, D + XR), BF16),
            pltpu.VMEM((D, H * HP), BF16),
            pltpu.VMEM((3 * D, D + XR), BF16),
            pltpu.VMEM((D, H * HP), BF16),
            pltpu.VMEM((NB * H, HP, TB), F32),
            pltpu.VMEM((NB * H, 5 * 16, TB // 2), F32),
            pltpu.VMEM((S // 2, HP), U32),
            pltpu.VMEM((NB, HP // 2, TB), U32),
            pltpu.VMEM((NB, H * HP, TB), BF16),
            pltpu.VMEM((NB, 8, TB), F32),
            pltpu.VMEM((NB, H, TB), F32),
            pltpu.VMEM((NB, H, TB), F32),
            pltpu.VMEM((NC * VK, HP), F32),
            pltpu.VMEM((8, TB), F32),
            pltpu.VMEM((KB0 + NC * 7 * HD * 8, CK), F32),
            pltpu.VMEM((UA * S, TB - CK), F32),
            pltpu.VMEM((H, S, CK), BF16),
            pltpu.VMEM((H, NC * HP, CK), BF16),
            pltpu.VMEM((H, NC, HP, CK), BF16),
        ],
        compiler_params=pltpu.CompilerParams(vmem_limit_bytes=100 * 2**20),
    )(A_x.reshape(S, D).T, A_wq, A_wk.T, A_wv.T, A_wo, B_wqkv, B_wo)
    return out_t.T.reshape(1, S, D)
```

```python
import jax
import jax.numpy as jnp
import numpy as np
from jax import lax
import jax.experimental.pallas as pl
import jax.experimental.pallas.tpu as pltpu

S, D, H, DH, WIN = 2048, 448, 16, 28, 256
HP = 32
HD = DH // 2
XR = 16
TB = 512
NB = S // TB
CK = 128
NC = S // CK
PER = TB // CK
MR = 64
UA = 4
UB = 4
VK = 16
LEAD = 20
STEPS = (12, 12, 11, 13, 12, 16, 22)
KB0 = max(UA, 2 * UB) * S
assert LEAD < 6 * HD and sum(STEPS) == 7 * HD and len(STEPS) * 16 == CK - VK
QSCALE = float(DH ** -0.5 * np.log2(np.e))
SUM_MIN, SUM_MAX = 2.0 ** -80, 2.0 * S
F32, BF16, U32 = jnp.float32, jnp.bfloat16, jnp.uint32


def _mm(a, b):
    return jnp.dot(a, b, preferred_element_type=F32)


def _merge(*streams):
    keyed = [((i + 0.5) / len(s), n, f) for n, s in enumerate(streams) for i, f in enumerate(s)]
    return [f for _, _, f in sorted(keyed, key=lambda e: e[:2])]


def _run(thunks):
    for f in thunks:
        f()


def _split_rows(v, parts):
    head = v.astype(BF16).astype(F32)
    row = lax.broadcasted_iota(jnp.int32, (XR, v.shape[1]), 0)
    out = jnp.zeros(row.shape, F32)
    for i, part in enumerate(parts):
        out = jnp.where(row == i, v - head if part else head, out)
    return out


def _with_column_sums(w):
    return jnp.concatenate([w, _split_rows(jnp.sum(w, axis=0, keepdims=True), (0, 1, 0))], axis=0)


def _key(b):
    return b if isinstance(b, int) else None


def _aligned(i, n):
    return i if isinstance(i, int) else pl.multiple_of(i, n)


def _kernel(xt_hbm, wq_hbm, wkt_hbm, wvt_hbm, wo_hbm, wqkv_hbm, bwo_hbm, out_hbm,
            h_s, wq_in, wkt_in, wvt_in, wo_in, wqkv_in, bwo_in, sems, zero_s,
            x_s, wa_s, woa_s, wb_s, wob_s, q_s, qf_s, ka_s, va_s, o_s, mean_s, qn_s, kn_s, kv_s, unsafe_s,
            pa_s, pb_s, kb_s, kr_s, vb_s):
    def x_copy(b):
        return pltpu.make_async_copy(
            xt_hbm.at[:, pl.ds(_aligned(b * TB, TB), TB)], h_s.at[b, pl.ds(0, D)], sems.at[b])

    def out_copy(b):
        return pltpu.make_async_copy(
            h_s.at[b, pl.ds(0, D)], out_hbm.at[:, pl.ds(_aligned(b * TB, TB), TB)], sems.at[b])

    def last_out_copy(r):
        return pltpu.make_async_copy(
            h_s.at[NB - 1, pl.ds(r * MR, MR)], out_hbm.at[pl.ds(r * MR, MR), pl.ds(S - TB, TB)], sems.at[NB + r])

    wk_copy, wv_copy, wq_copy, *later_copies = [
        pltpu.make_async_copy(src, dst, sems.at[NB + D // MR + i]) for i, (src, dst) in enumerate(
            [(wkt_hbm, wkt_in), (wvt_hbm, wvt_in), (wq_hbm, wq_in),
             (wo_hbm, wo_in), (wqkv_hbm, wqkv_in), (bwo_hbm, bwo_in)])]

    ones_row = jnp.where(lax.broadcasted_iota(jnp.int32, (HP, TB), 0) == DH, 1.0, 0.0).astype(F32)
    spare = lax.broadcasted_iota(jnp.int32, (8, TB), 0) == DH % 8
    lane = lax.broadcasted_iota(jnp.int32, (HP, CK), 1)
    causal = lax.broadcasted_iota(jnp.int32, (CK, CK), 0) <= lax.broadcasted_iota(jnp.int32, (CK, CK), 1)
    scale, stats = {}, {}

    def moments(b, d, first):
        d = d.reshape(d.shape[0] // 8, 8, d.shape[1])
        s1, s2 = jnp.sum(d, axis=0), jnp.sum(d * d, axis=0)
        stats[_key(b)] = (s1, s2) if first else (stats[_key(b)][0] + s1, stats[_key(b)][1] + s2)

    def layernorm(b, first=False):
        def piece():
            s1, s2 = stats[_key(b)]
            mean = jnp.sum(s1, axis=0, keepdims=True) * (1.0 / D)
            var = jnp.sum(s2, axis=0, keepdims=True) * (1.0 / D) - mean * mean
            scale[_key(b)] = lax.rsqrt(jnp.maximum(var, 0.0) + 1e-5)
            h_s[b, D:, :] = _split_rows(-mean, (0, 0, 1)).astype(BF16)
            mean_s[b] = jnp.broadcast_to(mean, (8, TB)) if first else mean_s[b] + mean
        return [piece]

    def input_layernorm(b):
        return [lambda r=r: moments(b, h_s[b, r * MR:(r + 1) * MR, :].astype(F32), r == 0)
                for r in range(D // MR)] + layernorm(b, True)

    def per_head(w_s, r0, b, factor, emit):
        ys = []

        def piece(j):
            y = _mm(w_s[r0 + j * MR:r0 + (j + 1) * MR, :], h_s[b])
            ys.append(y * (scale[_key(b)] * factor if factor else scale[_key(b)]))
            for h in range(H):
                if j * MR < (h + 1) * DH <= (j + 1) * MR:
                    j0 = h * DH // MR
                    rows = jnp.concatenate(ys[j0:], axis=0)[h * DH - j0 * MR:(h + 1) * DH - j0 * MR]
                    emit(h, jnp.concatenate([rows, jnp.zeros((HP - DH, TB), F32)], axis=0))
        return [lambda j=j: piece(j) for j in range(D // MR)]

    def put_q(b, factors=False):
        def emit(h, q):
            q_s[b * H + h] = q
            if factors:
                b11, b12, b21, b22 = (jnp.concatenate([x[:, c * CK:(c + 1) * CK] for c in (i, i + 2)], axis=1)
                                      for x in (q[0:16], q[HD:HD + 16]) for i in (0, 1))
                qf_s[b * H + h] = jnp.concatenate([b21 - b11, b11 + b22, b21 + b22, b12 - b22, b11 + b12], axis=0)
            qn_s[b, h:h + 1, :] = jnp.sum(q * q, axis=0, keepdims=True)
        return emit

    def a_proj(b):
        def kv():
            y = _mm(wa_s[D:D + 2 * HP, :], h_s[b]) * scale[_key(b)]
            kn_s[b, 0:1, :] = jnp.sum(y[0:HP] * y[0:HP], axis=0, keepdims=True)
            k = (y[0:HP] + ones_row).T
            ka_s[pl.ds(_aligned(b * (TB // 2), TB // 2), TB // 2), :] = pltpu.bitcast(k.astype(BF16), U32)
            va_s[b] = pltpu.bitcast((y[HP:2 * HP] + ones_row).astype(BF16), U32)
            for c in range(PER):
                kv_s[pl.ds(_aligned((b * PER + c) * VK, VK), VK), :] = k[(c + 1) * CK - VK:(c + 1) * CK]
        return [kv] + per_head(wa_s, 0, b, QSCALE, put_q(b, True))

    def b_proj(b):
        def put_k(h, k):
            kn_s[b, h:h + 1, :] = jnp.sum(k * k, axis=0, keepdims=True)
            k = k + ones_row
            for c in range(PER):
                kw = jnp.concatenate([k[:, c * CK:(c + 1) * CK]] * 4, axis=0).T
                parts = [jnp.where((lane >= g * HP) & (lane < (g + 1) * HP), kw[g * HP:(g + 1) * HP], 0.0)
                         for g in range(4)]
                t = b * PER + c
                kb_s[h, pl.ds(_aligned(t * CK, CK), CK), :] = jnp.concatenate(parts, axis=0).astype(BF16)
                kr_s[h, pl.ds(_aligned(t * HP, HP), HP), :] = (
                    (parts[0] + parts[1]) + (parts[2] + parts[3])).astype(BF16)

        def put_v(h, v):
            v = (v + ones_row).astype(BF16)
            for c in range(PER):
                vb_s[h, b * PER + c] = v[:, c * CK:(c + 1) * CK]
        return _merge(per_head(wb_s, D, b, None, put_k),
                      per_head(wb_s, 0, b, QSCALE, put_q(b)) + per_head(wb_s, 2 * D, b, None, put_v))

    def out_proj(w_s, b, first=False, last=False):
        def piece(r):
            rows = slice(r * MR, (r + 1) * MR)
            x = h_s[b, rows, :].astype(F32) if first else x_s[b, rows, :]
            x = x + _mm(w_s[rows, :], o_s[b])
            if last:
                h_s[b, rows, :] = x.astype(BF16)
            else:
                x_s[b, rows, :] = x
                d = (x.reshape(MR // 8, 8, TB) - mean_s[b]).reshape(MR, TB)
                h_s[b, rows, :] = d.astype(BF16)
                moments(b, d, r == 0)
        return [lambda r=r: piece(r) for r in range(D // MR)]

    def transposed(dst, src, pad_heads):
        def piece(c0, c1):
            w = src[:, c0:c1].astype(F32)
            if pad_heads:
                z = jnp.zeros((HP - DH, c1 - c0), F32)
                w = jnp.concatenate([p for h in range(H) for p in (w[h * DH:(h + 1) * DH], z)], axis=0)
            else:
                w = _with_column_sums(w)
            dst[c0:c1, :] = w.T.astype(BF16)
        n = src.shape[1]
        return [lambda c=c: piece(c, min(c + CK, n)) for c in range(0, n, CK)]

    def kv_weights():
        z = jnp.zeros((HP - DH, D), F32)
        w = jnp.concatenate([wkt_in[...].astype(F32), z, wvt_in[...].astype(F32), z], axis=0)
        wa_s[D:D + 2 * HP, :] = _with_column_sums(w.T).T.astype(BF16)

    def bound_scores(heads, order):
        k2 = jnp.max(jnp.max(kn_s[:, 0:heads, :], axis=0), axis=1, keepdims=True)
        shift = (-jnp.sqrt(qn_s[...] * k2)).astype(BF16).astype(F32)

        def piece(b, h):
            q_s[b * H + h, HP - 8:, :] = jnp.where(spare, shift[b, h:h + 1, :], q_s[b * H + h, HP - 8:, :])
        return [lambda b=b, h=h: piece(b, h) for b, h in order]

    def put_head(b, h, cols, o):
        o_s[b, pl.ds(_aligned(h * HP, HP), HP), cols] = o.astype(BF16)

    def finish(b, h, cols, acc):
        total = acc[HP - 8:]
        r = pl.reciprocal(total, approx=True)
        r = r * (2.0 - total * r)
        put_head(b, h, cols, acc * r[DH % 8:DH % 8 + 1])
        unsafe_s[:, cols] = jnp.where((total >= SUM_MIN) & (total <= SUM_MAX), unsafe_s[:, cols], 1.0)

    def key_rows(j, m, d, zero):
        r = KB0 + 8 * ((j * 7 + m) * HD + d)
        return slice(r, r + 8) if zero is None else pl.ds(pl.multiple_of(zero + r, 8), 8)

    def spread_keys():
        def piece(j, d):
            a11, a12, a21, a22 = (jnp.broadcast_to(kv_s[VK * j + r:VK * j + r + 8, i:i + 1], (8, CK))
                                  for r in (0, 8) for i in (d, HD + d))
            for m, a in enumerate((a22, a21 + a22, a11 + a22, a12 - a22, a11 + a12, a11, a21 - a11)):
                pa_s[key_rows(j, m, d, zero_s[0] if m == 0 else None), :] = a
        return [lambda j=j, d=d: piece(j, d) for j in range(NC) for d in range(HD)]

    def put_weights(r0, p):
        pa_s[r0:r0 + p.shape[0], :] = p[:, :CK]
        pb_s[r0:r0 + p.shape[0], :] = p[:, CK:]

    def a_values(t, u):
        st = {}

        def piece(c):
            rows = slice(u * S + c * CK, u * S + (c + 1) * CK)
            v = pltpu.bitcast(va_s[c // PER, :, (c % PER) * CK:(c % PER + 1) * CK], BF16)
            d = _mm(v, jnp.concatenate([pa_s[rows, :], pb_s[rows, :]], axis=1).astype(BF16))
            st["acc"] = d if c == 0 else st["acc"] + d
            if c == NC - 1:
                finish(t // H, t % H, slice(None), st["acc"])
        return [lambda c=c: piece(c) for c in range(NC)]

    def vector_scores(t, u):
        st = {}
        zero = zero_s[0]

        def piece(j, m, d, tied):
            k = pa_s[key_rows(j, m, d, zero if tied else None), :]
            for half in range(2):
                left, right = (slice(c * CK, (c + 1) * CK) for c in (2 * half, 2 * half + 1))
                if m == 1:
                    q = q_s[t, d:d + 1, left]
                elif m == 4:
                    q = q_s[t, HD + d:HD + d + 1, right]
                else:
                    i = 16 * (m - (m > 1) - (m > 4)) + d
                    q = qf_s[t, i:i + 1, half * CK:(half + 1) * CK]
                if d > 0:
                    st[half] = st[half] + k * q
                elif m in (0, 5):
                    st[half] = q_s[t, DH:DH + 1, left if m == 0 else right] + k * q
                else:
                    st[half] = k * q
                if d == HD - 1:
                    p, c = st[half], st.setdefault((j, half), {})
                    if m == 0:
                        c[11] = p
                    elif m == 1:
                        c[21], c[22] = c[11] + p, p
                    elif m == 2:
                        c[11], c[22] = c[11] + p, p - c[22]
                    elif m == 3:
                        c[11] = c[11] + p
                    elif m == 4:
                        c[11], c[12] = c[11] - p, p
                    elif m == 5:
                        c[12], c[22] = c[12] + p, c[22] + p
                    else:
                        c[22] = c[22] + p
            if d == HD - 1 and m >= 5:
                g = m - 5
                s = [st[j, half][10 * g + c] for half in range(2) for c in (11, 12)]
                put_weights(u * S + (j + 1) * CK - VK + 8 * g, jnp.exp2(jnp.concatenate(s, axis=1)))
        return [lambda tied, j=j, m=m, d=d: piece(j, m, d, tied)
                for j in range(NC) for m in range(7) for d in range(HD)]

    def a_weights(t, u, tick=None):
        st = {}

        def piece(c):
            if c == 0:
                st["q"] = q_s[t].astype(BF16)
            k0, k1 = c * CK, (c + 1) * CK - (VK if tick else 0)
            s = _mm(pltpu.bitcast(ka_s[k0 // 2:k1 // 2, :], BF16), st["q"])
            for r0 in range(k0, k1, 16):
                put_weights(u * S + r0, jnp.exp2(s[r0 - k0:r0 - k0 + 16]))
                if tick:
                    tick((r0 - k0) // 16)
        return [lambda c=c: piece(c) for c in range(NC)]

    def a_block(base, n_values, n_weights, fill=()):
        tick = None
        if n_values and n_weights:
            steps = [f for j in range(n_weights) for f in vector_scores(base + n_values + j, j)]
            lead = [LEAD]

            def tick(i):
                n = lead[0] + STEPS[i]
                for x, f in enumerate(steps[:n]):
                    y = x - lead[0]
                    f(y == 7 or (i == 6 and y == 15) or (y < 0 and x % 12 == 6))
                del steps[:n]
                lead[0] = 0
        values = [f for j in range(n_values) for f in a_values(base + j, j)]
        weights = [f for j in range(n_weights) for f in a_weights(base + n_values + j, j, tick)]
        _run(_merge(values, weights, list(fill)))

    def a_exact(t, _):
        q = q_s[t].astype(BF16)

        def scores(j):
            return _mm(pltpu.bitcast(ka_s[pl.ds(pl.multiple_of(j * (TB // 2), TB // 2), TB // 2), :], BF16), q)
        m = lax.fori_loop(0, NB, lambda j, m: jnp.maximum(m, jnp.max(scores(j), axis=0, keepdims=True)),
                          jnp.full((1, TB), -jnp.inf, F32))
        acc = lax.fori_loop(0, NB, lambda j, acc: acc + _mm(
            pltpu.bitcast(va_s[j], BF16), jnp.exp2(scores(j) - m).astype(BF16)), jnp.zeros((HP, TB), F32))
        put_head(t // H, t % H, slice(None), acc / acc[DH:DH + 1])
        return _

    def b_step(h0, u, do_values, do_weights):
        st = {}

        def by_group(right, left):
            parts = [right[0:HP]]
            for g in range(1, 4):
                rows = slice(g * HP, (g + 1) * HP)
                parts.append(jnp.where(lane >= g * HP, right[rows], left[rows]))
            return jnp.concatenate(parts, axis=0)

        def weights(i):
            h = h0 + UB if do_values else h0
            q0, q1 = (q_s[j // PER * H + h, :, j % PER * CK:(j % PER + 1) * CK] for j in (i, min(i + 1, NC - 1)))
            w = jnp.concatenate([q0] + [jnp.where(lane >= g * HP, q0, q1) for g in range(1, 4)], axis=0).astype(BF16)
            before = _mm(kb_s[h, (i - 1) * CK:i * CK, :], w) if i >= 1 else None
            same = _mm(kb_s[h, i * CK:(i + 1) * CK, :], w)
            if i >= 2:
                wr = jnp.concatenate([jnp.where((lane >= g * HP) & (lane < (g + 1) * HP), q0, 0.0)
                                      for g in range(4)], axis=0)
                r = _mm(kr_s[h, (i - 2) * HP:(i - 1) * HP, :], wr.astype(BF16))
                oldest = by_group(jnp.concatenate([r] * 4, axis=0), st["before"])
            else:
                oldest = -jnp.inf
            r0 = (u * NC + i) * 2 * CK
            pa_s[r0:r0 + CK, :] = jnp.exp2(jnp.where(causal, same, oldest))
            if i >= 1:
                pa_s[r0 + CK:r0 + 2 * CK, :] = jnp.exp2(by_group(before, st["same"]))
            st["same"], st["before"] = same, before

        def values(i):
            r0 = (u * NC + i) * 2 * CK
            edge = pa_s[r0:r0 + CK, :]
            acc = _mm(vb_s[h0, i], jnp.where(causal, edge, 0.0).astype(BF16))
            if i >= 1:
                acc += _mm(vb_s[h0, i - 1], pa_s[r0 + CK:r0 + 2 * CK, :].astype(BF16))
            if i >= 2:
                acc += _mm(vb_s[h0, i - 2], jnp.where(causal, 0.0, edge).astype(BF16))
            finish(i // PER, h0, slice(i % PER * CK, (i % PER + 1) * CK), acc)
        fs = ([values] if do_values else []) + ([weights] if do_weights else [])
        return [lambda f=f, i=i: f(i) for i in range(NC) for f in fs]

    def b_exact(t, _):
        b, h = t // H, t % H
        for c in range(PER):
            cols = slice(c * CK, (c + 1) * CK)
            j0 = jnp.maximum(b * PER + c - 2, 0)
            s = _mm(kb_s[h, pl.ds(pl.multiple_of(j0 * CK, CK), 3 * CK), :],
                    jnp.concatenate([q_s[t, :, cols]] * 4, axis=0).astype(BF16))
            age = ((b * PER + c - j0) * CK + lax.broadcasted_iota(jnp.int32, s.shape, 1)
                   - lax.broadcasted_iota(jnp.int32, s.shape, 0))
            s = jnp.where((age >= 0) & (age < WIN), s, -jnp.inf)
            p = jnp.exp2(s - jnp.max(s, axis=0, keepdims=True)).astype(BF16)
            acc = sum(_mm(vb_s[h, j0 + j], p[j * CK:(j + 1) * CK]) for j in range(3))
            put_head(b, h, cols, acc / acc[DH:DH + 1])
        return _

    zero_s[0] = 0
    unsafe_s[...] = jnp.zeros(unsafe_s.shape, F32)

    for cp in [wk_copy, wv_copy, x_copy(0), wq_copy] + [x_copy(b) for b in range(1, NB)] + later_copies:
        cp.start()
    wq_t, p0, p1 = transposed(wa_s, wq_in, False), a_proj(0), a_proj(1)
    wk_copy.wait()
    wv_copy.wait()
    kv_weights()
    x_copy(0).wait()
    _run(input_layernorm(0) + p0[:1])
    wq_copy.wait()
    _run([wq_t[0], wq_t[1], p0[1], wq_t[2], p0[2], wq_t[3], p0[3]])
    x_copy(1).wait()
    _run(_merge(p0[4:], input_layernorm(1)) + p1[:4])
    x_copy(2).wait()
    x_copy(3).wait()
    _run(_merge(p1[4:], input_layernorm(2)))
    _run(_merge(a_proj(2), input_layernorm(3)))
    _run(a_proj(3))

    for first in (True, False):
        bounds = bound_scores(1, [divmod(t, H) for t in range(NB * H)])
        _run(bounds[:UA])
        a_block(0, 0, UA, _merge(bounds[UA:], spread_keys()))
        if first:
            for cp in later_copies:
                cp.wait()
        lax.fori_loop(0, NB * H // UA - 1, lambda i, _: a_block(i * UA, UA, UA), None)
        a_block(NB * H - UA, UA, 0, transposed(woa_s, wo_in, True) if first else ())

        out = [f for b in range(NB) for f in out_proj(woa_s, b, first=first) + layernorm(b)]
        _run(_merge(out, transposed(wb_s, wqkv_in, False) if first else []))
        _run(b_proj(0) + b_proj(1) + b_proj(2))
        _run(_merge(b_proj(3), transposed(wob_s, bwo_in, True) if first else []))

        bounds = bound_scores(H, [(b, h) for h in range(H) for b in range(NB)])
        _run(bounds[:NB])
        _run(_merge([f for u in range(UB) for f in b_step(u, u, False, True)], bounds[NB:]))
        lax.fori_loop(0, H // UB - 1,
                      lambda i, _: _run([f for u in range(UB) for f in b_step(i * UB + u, u, True, True)]), None)
        _run([f for u in range(UB) for f in b_step(H - UB + u, u, True, False)])

        if first:
            _run([f for b in range(NB) for f in out_proj(wob_s, b) + layernorm(b)])
            _run([f for b in range(NB) for f in a_proj(b)])

    for b in range(NB - 1):
        _run(out_proj(wob_s, b, last=True))
        out_copy(b).start()
    for r, f in enumerate(out_proj(wob_s, NB - 1, last=True)):
        f()
        last_out_copy(r).start()
    unsafe = jnp.max(jnp.where(spare, unsafe_s[...], 0.0)) > 0.0
    for b in range(NB - 1):
        out_copy(b).wait()
    for r in range(D // MR):
        last_out_copy(r).wait()

    @pl.when(unsafe)
    def _():
        def blocks(stages):
            lax.fori_loop(0, NB, lambda b, _: _run(stages(b)), None)

        def reload(b):
            x_copy(b).start()
            x_copy(b).wait()
            x_s[b] = h_s[b, 0:D, :].astype(F32)
            return input_layernorm(b) + a_proj(b)

        def layer_pair(r, _):
            lax.fori_loop(0, NB * H, a_exact, None)
            blocks(lambda b: out_proj(woa_s, b) + layernorm(b) + b_proj(b))
            lax.fori_loop(0, NB * H, b_exact, None)
            blocks(lambda b: out_proj(wob_s, b) + layernorm(b) + a_proj(b))

        def store(b, _):
            h_s[b, 0:D, :] = x_s[b].astype(BF16)
            out_copy(b).start()
            out_copy(b).wait()
        blocks(reload)
        lax.fori_loop(0, 2, layer_pair, None)
        lax.fori_loop(0, NB, store, None)


@jax.jit
def pallas_interleave_layers__grouped_kv_mqa__sliding_block__prompt_kernel(
    A_x: jax.Array,
    A_wq: jax.Array,
    A_wk: jax.Array,
    A_wv: jax.Array,
    A_wo: jax.Array,
    B_x: jax.Array,
    B_wqkv: jax.Array,
    B_wo: jax.Array,
):
    del B_x
    out_t = pl.pallas_call(
        _kernel,
        out_shape=jax.ShapeDtypeStruct((D, S), BF16),
        in_specs=[pl.BlockSpec(memory_space=pl.ANY)] * 7,
        out_specs=pl.BlockSpec(memory_space=pl.ANY),
        scratch_shapes=[
            pltpu.VMEM((NB, D + XR, TB), BF16),
            pltpu.VMEM((D, D), BF16),
            pltpu.VMEM((DH, D), BF16),
            pltpu.VMEM((DH, D), BF16),
            pltpu.VMEM((D, D), BF16),
            pltpu.VMEM((D, 3 * D), BF16),
            pltpu.VMEM((D, D), BF16),
            pltpu.SemaphoreType.DMA((NB + D // MR + 6,)),
            pltpu.SMEM((1,), jnp.int32),
            pltpu.VMEM((NB, D, TB), F32),
            pltpu.VMEM((D + 2 * HP, D + XR), BF16),
            pltpu.VMEM((D, H * HP), BF16),
            pltpu.VMEM((3 * D, D + XR), BF16),
            pltpu.VMEM((D, H * HP), BF16),
            pltpu.VMEM((NB * H, HP, TB), F32),
            pltpu.VMEM((NB * H, 5 * 16, TB // 2), F32),
            pltpu.VMEM((S // 2, HP), U32),
            pltpu.VMEM((NB, HP // 2, TB), U32),
            pltpu.VMEM((NB, H * HP, TB), BF16),
            pltpu.VMEM((NB, 8, TB), F32),
            pltpu.VMEM((NB, H, TB), F32),
            pltpu.VMEM((NB, H, TB), F32),
            pltpu.VMEM((NC * VK, HP), F32),
            pltpu.VMEM((8, TB), F32),
            pltpu.VMEM((KB0 + NC * 7 * HD * 8, CK), F32),
            pltpu.VMEM((UA * S, TB - CK), F32),
            pltpu.VMEM((H, S, CK), BF16),
            pltpu.VMEM((H, NC * HP, CK), BF16),
            pltpu.VMEM((H, NC, HP, CK), BF16),
        ],
        compiler_params=pltpu.CompilerParams(vmem_limit_bytes=100 * 2**20),
    )(A_x.reshape(S, D).T, A_wq, A_wk.T, A_wv.T, A_wo, B_wqkv, B_wo)
    return out_t.T.reshape(1, S, D)
```
